```python
import os as _os
_os.environ.setdefault("JAX_PLATFORMS", "cpu")
import jax
import jax.numpy as jnp

def _softmax(x, axis=-1):
    return jax.nn.softmax(x, axis=axis)
def _gelu(x):
    return jax.nn.gelu(x, approximate=True)
def _silu(x):
    return jax.nn.silu(x)
def _sigmoid(x):
    return jax.nn.sigmoid(x)
def _layernorm(x, axis=-1, eps=1e-5):
    m = jnp.mean(x, axis=axis, keepdims=True)
    v = jnp.var(x, axis=axis, keepdims=True)
    return (x - m) / jnp.sqrt(v + eps)
def _scatter_add(tgt, idx, src, axis=0):
    return tgt.at[idx].add(src)
def _segment_sum(src, seg, n):
    return jax.ops.segment_sum(src, seg, n)
class _Rng:
    def __init__(self, key):
        self._k = key
    def _next(self):
        self._k, sub = jax.random.split(self._k)
        return sub
    def normal(self, shape):
        return jax.random.normal(self._next(), shape, dtype=jnp.bfloat16)
    def randint(self, lo, hi, shape):
        return jax.random.randint(self._next(), shape, lo, hi, dtype=jnp.int32)
    def uniform(self, shape, lo=0.0, hi=1.0):
        return jax.random.uniform(self._next(), shape, jnp.bfloat16, lo, hi)
    def permutation(self, n):
        return jax.random.permutation(self._next(), n)


kernel_name = 'concat_heads__gqa_block_cached__gqa_block_cached__near_ridge'

def setup_inputs():
    _rng = _Rng(jax.random.key(int.from_bytes(__import__("os").urandom(4), "little")))
    _w = (lambda a: (lambda t: t.astype(jnp.bfloat16) if jnp.issubdtype(t.dtype, jnp.floating) else t)(jnp.asarray(a)))
    def _A_setup():
        B, Sq, D = 8, 240, 640
        Hq, Hkv, Sk, Dh = 32, 32, 1024, 192
        assert Hq % Hkv == 0, (Hq, Hkv)
        return {
            "x": _w((lambda *s: _rng.normal(s) * 0.8)(B, Sq, D)),
            "k_cache": _w((lambda *s: _rng.normal(s) * 0.8)(B, Hkv, Sk, Dh)),
            "v_cache": _w((lambda *s: _rng.normal(s) * 0.05)(B, Hkv, Sk, Dh)),
            "wq": _w((lambda *s: _rng.normal(s) * 0.8)(D, Hq * Dh) * (D ** -0.5)),
            "wo": _w((lambda *s: _rng.normal(s) * 0.05)(Hq * Dh, D) * ((Hq * Dh) ** -0.5)),
        }
    _A_in = _A_setup()

    def _B_setup():
        B, Sq, D = 8, 240, 640
        Hq, Hkv, Sk, Dh = 32, 32, 1024, 192
        assert Hq % Hkv == 0, (Hq, Hkv)
        return {
            "x": _w((lambda *s: _rng.normal(s) * 0.8)(B, Sq, D)),
            "k_cache": _w((lambda *s: _rng.normal(s) * 0.8)(B, Hkv, Sk, Dh)),
            "v_cache": _w((lambda *s: _rng.normal(s) * 0.05)(B, Hkv, Sk, Dh)),
            "wq": _w((lambda *s: _rng.normal(s) * 0.8)(D, Hq * Dh) * (D ** -0.5)),
            "wo": _w((lambda *s: _rng.normal(s) * 0.05)(Hq * Dh, D) * ((Hq * Dh) ** -0.5)),
        }
    _B_in = _B_setup()

    return {
        "A_x": _A_in["x"],
        "A_k_cache": _A_in["k_cache"],
        "A_v_cache": _A_in["v_cache"],
        "A_wq": _A_in["wq"],
        "A_wo": _A_in["wo"],
        "B_x": _B_in["x"],
        "B_k_cache": _B_in["k_cache"],
        "B_v_cache": _B_in["v_cache"],
        "B_wq": _B_in["wq"],
        "B_wo": _B_in["wo"],
    }

def reference(A_x, A_k_cache, A_v_cache, A_wq, A_wo, B_x, B_k_cache, B_v_cache, B_wq, B_wo):
    def _A_ref(x, k_cache, v_cache, wq, wo):
        B, Sq, D = x.shape
        Hq, Dh = 32, 192
        Hkv = k_cache.shape[1]
        rep = Hq // Hkv
        q = (lambda x, *d: x.transpose(*d))((x @ wq).reshape(B, Sq, Hq, Dh), 0, 2, 1, 3)
        k = jnp.repeat(k_cache, rep, axis=1)
        v = jnp.repeat(v_cache, rep, axis=1)
        scores = jnp.einsum("bhqd,bhkd->bhqk", q, k) * (Dh ** -0.5)
        p = _softmax(scores, axis=-1)
        o = jnp.einsum("bhqk,bhkd->bhqd", p, v)
        return (lambda x, *d: x.transpose(*d))(o, 0, 2, 1, 3).reshape(B, Sq, Hq * Dh) @ wo

    def _B_ref(x, k_cache, v_cache, wq, wo):
        B, Sq, D = x.shape
        Hq, Dh = 32, 192
        Hkv = k_cache.shape[1]
        rep = Hq // Hkv
        q = (lambda x, *d: x.transpose(*d))((x @ wq).reshape(B, Sq, Hq, Dh), 0, 2, 1, 3)
        k = jnp.repeat(k_cache, rep, axis=1)
        v = jnp.repeat(v_cache, rep, axis=1)
        scores = jnp.einsum("bhqd,bhkd->bhqk", q, k) * (Dh ** -0.5)
        p = _softmax(scores, axis=-1)
        o = jnp.einsum("bhqk,bhkd->bhqd", p, v)
        return (lambda x, *d: x.transpose(*d))(o, 0, 2, 1, 3).reshape(B, Sq, Hq * Dh) @ wo

    a = _A_ref(A_x, A_k_cache, A_v_cache, A_wq, A_wo)
    b = _B_ref(B_x, B_k_cache, B_v_cache, B_wq, B_wo)
    return jnp.concatenate([a, b], axis=-1)
```

```python
import functools

import jax
import jax.numpy as jnp
import jax.experimental.pallas as pl
import jax.experimental.pallas.tpu as pltpu

HPS = 2


def _attend(q, k, v):
    s = jax.lax.dot_general(
        q, k, (((1,), (1,)), ((), ())), preferred_element_type=jnp.float32
    )
    m = jnp.max(s, axis=-1, keepdims=True)
    p = jnp.exp(s - m)
    l = jnp.sum(p, axis=-1, keepdims=True)
    o = jnp.dot(p.astype(jnp.bfloat16), v, preferred_element_type=jnp.float32)
    return o * (1.0 / l)


def _kernel(xa_ref, ka_ref, va_ref, wqa_ref, woa_ref,
            xb_ref, kb_ref, vb_ref, wqb_ref, wob_ref,
            o_ref, acc_ref, *, dh, d, scale):
    h = pl.program_id(1)
    nh = pl.num_programs(1)
    w = HPS * dh

    @pl.when(h == 0)
    def _():
        acc_ref[...] = jnp.zeros_like(acc_ref)

    off = pl.multiple_of(h * w, 128)
    for blk, (x_ref, k_ref, v_ref, wq_ref, wo_ref) in enumerate(
        ((xa_ref, ka_ref, va_ref, wqa_ref, woa_ref),
         (xb_ref, kb_ref, vb_ref, wqb_ref, wob_ref))
    ):
        x = x_ref[0]
        q2 = jnp.dot(x, wq_ref[:, pl.ds(off, w)], preferred_element_type=jnp.float32)
        q2 = (q2 * scale).astype(jnp.bfloat16)
        os = []
        for j in range(HPS):
            q = q2[:, j * dh:(j + 1) * dh]
            os.append(_attend(q, k_ref[0, j], v_ref[0, j]).astype(jnp.bfloat16))
        o2 = jnp.concatenate(os, axis=-1)
        y = jnp.dot(o2, wo_ref[pl.ds(off, w), :], preferred_element_type=jnp.float32)
        acc_ref[:, blk * d:(blk + 1) * d] += y

    @pl.when(h == nh - 1)
    def _():
        o_ref[0] = acc_ref[...].astype(o_ref.dtype)


@jax.jit
def pallas_concat_heads__gqa_block_cached__gqa_block_cached__near_ridge_kernel(
    A_x: jax.Array,
    A_k_cache: jax.Array,
    A_v_cache: jax.Array,
    A_wq: jax.Array,
    A_wo: jax.Array,
    B_x: jax.Array,
    B_k_cache: jax.Array,
    B_v_cache: jax.Array,
    B_wq: jax.Array,
    B_wo: jax.Array,
):
    B, Sq, D = A_x.shape
    _, H, Sk, Dh = A_k_cache.shape
    scale = float(Dh) ** -0.5

    x_spec = pl.BlockSpec((1, Sq, D), lambda b, h: (b, 0, 0))
    kv_spec = pl.BlockSpec((1, HPS, Sk, Dh), lambda b, h: (b, h, 0, 0))
    wq_spec = pl.BlockSpec((D, H * Dh), lambda b, h: (0, 0),
                           pipeline_mode=pl.Buffered(1))
    wo_spec = pl.BlockSpec((H * Dh, D), lambda b, h: (0, 0),
                           pipeline_mode=pl.Buffered(1))
    specs = [x_spec, kv_spec, kv_spec, wq_spec, wo_spec]

    return pl.pallas_call(
        functools.partial(_kernel, dh=Dh, d=D, scale=scale),
        grid=(B, H // HPS),
        in_specs=specs + specs,
        out_specs=pl.BlockSpec((1, Sq, 2 * D), lambda b, h: (b, 0, 0)),
        out_shape=jax.ShapeDtypeStruct((B, Sq, 2 * D), jnp.bfloat16),
        scratch_shapes=[pltpu.VMEM((Sq, 2 * D), jnp.float32)],
        compiler_params=pltpu.CompilerParams(
            dimension_semantics=("arbitrary", "arbitrary"),
            vmem_limit_bytes=100 * 1024 * 1024,
        ),
    )(A_x, A_k_cache, A_v_cache, A_wq, A_wo,
      B_x, B_k_cache, B_v_cache, B_wq, B_wo)
```

```python
import functools

import jax
import jax.numpy as jnp
import jax.experimental.pallas as pl
import jax.experimental.pallas.tpu as pltpu

HPS = 8


def _t(a):
    return jnp.swapaxes(a, 2, 3)


def _attend(q, k, v):
    s = jnp.dot(q, k, preferred_element_type=jnp.float32)
    m = jnp.max(s, axis=-1, keepdims=True)
    p = jnp.exp(s - m)
    l = jnp.sum(p, axis=-1, keepdims=True)
    o = jax.lax.dot_general(
        p.astype(jnp.bfloat16), v, (((1,), (1,)), ((), ())),
        preferred_element_type=jnp.float32,
    )
    return o * (1.0 / l)


def _kernel(xa_ref, ka_ref, va_ref, wqa_ref, woa_ref,
            xb_ref, kb_ref, vb_ref, wqb_ref, wob_ref,
            o_ref, acc_ref, *, dh, d, scale):
    h = pl.program_id(1)
    nh = pl.num_programs(1)
    w = HPS * dh

    @pl.when(h == 0)
    def _():
        acc_ref[...] = jnp.zeros_like(acc_ref)

    off = pl.multiple_of(h * w, 128)
    for blk, (x_ref, k_ref, v_ref, wq_ref, wo_ref) in enumerate(
        ((xa_ref, ka_ref, va_ref, wqa_ref, woa_ref),
         (xb_ref, kb_ref, vb_ref, wqb_ref, wob_ref))
    ):
        x = x_ref[0]
        q2 = jnp.dot(x, wq_ref[:, pl.ds(off, w)], preferred_element_type=jnp.float32)
        q2 = (q2 * scale).astype(jnp.bfloat16)
        os = []
        for j in range(HPS):
            q = q2[:, j * dh:(j + 1) * dh]
            os.append(_attend(q, k_ref[0, j], v_ref[0, j]).astype(jnp.bfloat16))
        o2 = jnp.concatenate(os, axis=-1)
        y = jnp.dot(o2, wo_ref[pl.ds(off, w), :], preferred_element_type=jnp.float32)
        acc_ref[:, blk * d:(blk + 1) * d] += y

    @pl.when(h == nh - 1)
    def _():
        o_ref[0] = acc_ref[...].astype(o_ref.dtype)


@jax.jit
def pallas_concat_heads__gqa_block_cached__gqa_block_cached__near_ridge_kernel(
    A_x: jax.Array,
    A_k_cache: jax.Array,
    A_v_cache: jax.Array,
    A_wq: jax.Array,
    A_wo: jax.Array,
    B_x: jax.Array,
    B_k_cache: jax.Array,
    B_v_cache: jax.Array,
    B_wq: jax.Array,
    B_wo: jax.Array,
):
    B, Sq, D = A_x.shape
    _, H, Sk, Dh = A_k_cache.shape
    scale = float(Dh) ** -0.5

    x_spec = pl.BlockSpec((1, Sq, D), lambda b, h: (b, 0, 0))
    kv_spec = pl.BlockSpec((1, HPS, Dh, Sk), lambda b, h: (b, h, 0, 0))
    wq_spec = pl.BlockSpec((D, H * Dh), lambda b, h: (0, 0),
                           pipeline_mode=pl.Buffered(1))
    wo_spec = pl.BlockSpec((H * Dh, D), lambda b, h: (0, 0),
                           pipeline_mode=pl.Buffered(1))
    specs = [x_spec, kv_spec, kv_spec, wq_spec, wo_spec]

    return pl.pallas_call(
        functools.partial(_kernel, dh=Dh, d=D, scale=scale),
        grid=(B, H // HPS),
        in_specs=specs + specs,
        out_specs=pl.BlockSpec((1, Sq, 2 * D), lambda b, h: (b, 0, 0)),
        out_shape=jax.ShapeDtypeStruct((B, Sq, 2 * D), jnp.bfloat16),
        scratch_shapes=[pltpu.VMEM((Sq, 2 * D), jnp.float32)],
        compiler_params=pltpu.CompilerParams(
            dimension_semantics=("arbitrary", "arbitrary"),
            vmem_limit_bytes=100 * 1024 * 1024,
        ),
    )(A_x, _t(A_k_cache), _t(A_v_cache), A_wq, A_wo,
      B_x, _t(B_k_cache), _t(B_v_cache), B_wq, B_wo)
```

```python
import functools

import jax
import jax.numpy as jnp
import jax.experimental.pallas as pl
import jax.experimental.pallas.tpu as pltpu

HPS = 4


def _t(a):
    return jnp.swapaxes(a, 2, 3)


def _qk(q, kt):
    return jnp.dot(q, kt, preferred_element_type=jnp.float32)


def _softmax_pv(s, vt):
    m = jnp.max(s, axis=-1, keepdims=True)
    p = jnp.exp2(s - m)
    l = jnp.sum(p, axis=-1, keepdims=True)
    o = jax.lax.dot_general(
        p.astype(jnp.bfloat16), vt, (((1,), (1,)), ((), ())),
        preferred_element_type=jnp.float32,
    )
    return (o * (1.0 / l)).astype(jnp.bfloat16)


def _kernel(xa_ref, ka_ref, va_ref, wqa_ref, woa_ref,
            xb_ref, kb_ref, vb_ref, wqb_ref, wob_ref,
            o_ref, acc_ref, *, dh, d, scale):
    h = pl.program_id(1)
    nh = pl.num_programs(1)
    w = HPS * dh

    @pl.when(h == 0)
    def _():
        acc_ref[...] = jnp.zeros_like(acc_ref)

    off = pl.multiple_of(h * w, 128)
    blocks = ((xa_ref, ka_ref, va_ref, wqa_ref, woa_ref),
              (xb_ref, kb_ref, vb_ref, wqb_ref, wob_ref))
    qs = []
    for (x_ref, k_ref, v_ref, wq_ref, wo_ref) in blocks:
        q2 = jnp.dot(x_ref[0], wq_ref[:, pl.ds(off, w)],
                     preferred_element_type=jnp.float32)
        qs.append((q2 * scale).astype(jnp.bfloat16))

    chains = [(blk, j) for blk in range(2) for j in range(HPS)]

    def qk(c):
        blk, j = chains[c]
        return _qk(qs[blk][:, j * dh:(j + 1) * dh], blocks[blk][1][0, j])

    os = [[], []]
    s_next = qk(0)
    for c, (blk, j) in enumerate(chains):
        s = s_next
        if c + 1 < len(chains):
            s_next = qk(c + 1)
        os[blk].append(_softmax_pv(s, blocks[blk][2][0, j]))
        if j == HPS - 1:
            o2 = jnp.concatenate(os[blk], axis=-1)
            y = jnp.dot(o2, blocks[blk][4][pl.ds(off, w), :],
                        preferred_element_type=jnp.float32)
            acc_ref[:, blk * d:(blk + 1) * d] += y

    @pl.when(h == nh - 1)
    def _():
        o_ref[0] = acc_ref[...].astype(o_ref.dtype)


@jax.jit
def pallas_concat_heads__gqa_block_cached__gqa_block_cached__near_ridge_kernel(
    A_x: jax.Array,
    A_k_cache: jax.Array,
    A_v_cache: jax.Array,
    A_wq: jax.Array,
    A_wo: jax.Array,
    B_x: jax.Array,
    B_k_cache: jax.Array,
    B_v_cache: jax.Array,
    B_wq: jax.Array,
    B_wo: jax.Array,
):
    B, Sq, D = A_x.shape
    _, H, Sk, Dh = A_k_cache.shape
    scale = float(Dh) ** -0.5 * 1.4426950408889634

    x_spec = pl.BlockSpec((1, Sq, D), lambda b, h: (b, 0, 0))
    kv_spec = pl.BlockSpec((1, HPS, Dh, Sk), lambda b, h: (b, h, 0, 0))
    wq_spec = pl.BlockSpec((D, H * Dh), lambda b, h: (0, 0),
                           pipeline_mode=pl.Buffered(1))
    wo_spec = pl.BlockSpec((H * Dh, D), lambda b, h: (0, 0),
                           pipeline_mode=pl.Buffered(1))
    specs = [x_spec, kv_spec, kv_spec, wq_spec, wo_spec]

    return pl.pallas_call(
        functools.partial(_kernel, dh=Dh, d=D, scale=scale),
        grid=(B, H // HPS),
        in_specs=specs + specs,
        out_specs=pl.BlockSpec((1, Sq, 2 * D), lambda b, h: (b, 0, 0)),
        out_shape=jax.ShapeDtypeStruct((B, Sq, 2 * D), jnp.bfloat16),
        scratch_shapes=[pltpu.VMEM((Sq, 2 * D), jnp.float32)],
        compiler_params=pltpu.CompilerParams(
            dimension_semantics=("arbitrary", "arbitrary"),
            vmem_limit_bytes=100 * 1024 * 1024,
        ),
    )(A_x, _t(A_k_cache), _t(A_v_cache), A_wq, A_wo,
      B_x, _t(B_k_cache), _t(B_v_cache), B_wq, B_wo)
```

```python
import functools

import jax
import jax.numpy as jnp
import jax.experimental.pallas as pl
import jax.experimental.pallas.tpu as pltpu

HPS = 8


def _t(a):
    return jnp.swapaxes(a, 2, 3)


def _qk(q, kt):
    return jnp.dot(q, kt, preferred_element_type=jnp.float32)


def _softmax_pv(s, vt):
    m = jnp.max(s, axis=-1, keepdims=True)
    p = jnp.exp2(s - m)
    l = jnp.sum(p, axis=-1, keepdims=True)
    o = jax.lax.dot_general(
        p.astype(jnp.bfloat16), vt, (((1,), (1,)), ((), ())),
        preferred_element_type=jnp.float32,
    )
    return (o * (1.0 / l)).astype(jnp.bfloat16)


def _kernel(xa_ref, ka_ref, va_ref, wqa_hbm, woa_hbm,
            xb_ref, kb_ref, vb_ref, wqb_hbm, wob_hbm,
            o_ref, acc_ref, wqa_ref, woa_ref, wqb_ref, wob_ref, sems,
            *, dh, d, scale, nh):
    b = pl.program_id(0)
    h = pl.program_id(1)
    w = HPS * dh

    def w_copies(i):
        cols = pl.ds(i * w, w)
        return [
            pltpu.make_async_copy(wqa_hbm.at[:, cols], wqa_ref.at[:, cols], sems.at[0, i]),
            pltpu.make_async_copy(wqb_hbm.at[:, cols], wqb_ref.at[:, cols], sems.at[1, i]),
            pltpu.make_async_copy(woa_hbm.at[cols, :], woa_ref.at[cols, :], sems.at[2, i]),
            pltpu.make_async_copy(wob_hbm.at[cols, :], wob_ref.at[cols, :], sems.at[3, i]),
        ]

    @pl.when(jnp.logical_and(b == 0, h == 0))
    def _():
        for i in range(nh):
            for cp in w_copies(i):
                cp.start()

    @pl.when(h == 0)
    def _():
        acc_ref[...] = jnp.zeros_like(acc_ref)

    for i in range(nh):
        @pl.when(jnp.logical_and(b == 0, h == i))
        def _():
            for cp in w_copies(i):
                cp.wait()

    off = pl.multiple_of(h * w, 128)
    blocks = ((xa_ref, ka_ref, va_ref, wqa_ref, woa_ref),
              (xb_ref, kb_ref, vb_ref, wqb_ref, wob_ref))
    qs = []
    for (x_ref, k_ref, v_ref, wq_ref, wo_ref) in blocks:
        q2 = jnp.dot(x_ref[0], wq_ref[:, pl.ds(off, w)],
                     preferred_element_type=jnp.float32)
        qs.append((q2 * scale).astype(jnp.bfloat16))

    chains = [(blk, j) for blk in range(2) for j in range(HPS)]

    def qk(c):
        blk, j = chains[c]
        return _qk(qs[blk][:, j * dh:(j + 1) * dh], blocks[blk][1][0, j])

    os = [[], []]
    s_next = qk(0)
    for c, (blk, j) in enumerate(chains):
        s = s_next
        if c + 1 < len(chains):
            s_next = qk(c + 1)
        os[blk].append(_softmax_pv(s, blocks[blk][2][0, j]))
        if j == HPS - 1:
            o2 = jnp.concatenate(os[blk], axis=-1)
            y = jnp.dot(o2, blocks[blk][4][pl.ds(off, w), :],
                        preferred_element_type=jnp.float32)
            acc_ref[:, blk * d:(blk + 1) * d] += y

    @pl.when(h == nh - 1)
    def _():
        o_ref[0] = acc_ref[...].astype(o_ref.dtype)


@jax.jit
def pallas_concat_heads__gqa_block_cached__gqa_block_cached__near_ridge_kernel(
    A_x: jax.Array,
    A_k_cache: jax.Array,
    A_v_cache: jax.Array,
    A_wq: jax.Array,
    A_wo: jax.Array,
    B_x: jax.Array,
    B_k_cache: jax.Array,
    B_v_cache: jax.Array,
    B_wq: jax.Array,
    B_wo: jax.Array,
):
    B, Sq, D = A_x.shape
    _, H, Sk, Dh = A_k_cache.shape
    nh = H // HPS
    scale = float(Dh) ** -0.5 * 1.4426950408889634

    x_spec = pl.BlockSpec((1, Sq, D), lambda b, h: (b, 0, 0))
    kv_spec = pl.BlockSpec((1, HPS, Dh, Sk), lambda b, h: (b, h, 0, 0))
    w_spec = pl.BlockSpec(memory_space=pl.ANY)
    specs = [x_spec, kv_spec, kv_spec, w_spec, w_spec]

    return pl.pallas_call(
        functools.partial(_kernel, dh=Dh, d=D, scale=scale, nh=nh),
        grid=(B, nh),
        in_specs=specs + specs,
        out_specs=pl.BlockSpec((1, Sq, 2 * D), lambda b, h: (b, 0, 0)),
        out_shape=jax.ShapeDtypeStruct((B, Sq, 2 * D), jnp.bfloat16),
        scratch_shapes=[
            pltpu.VMEM((Sq, 2 * D), jnp.float32),
            pltpu.VMEM((D, H * Dh), jnp.bfloat16),
            pltpu.VMEM((H * Dh, D), jnp.bfloat16),
            pltpu.VMEM((D, H * Dh), jnp.bfloat16),
            pltpu.VMEM((H * Dh, D), jnp.bfloat16),
            pltpu.SemaphoreType.DMA((4, nh)),
        ],
        compiler_params=pltpu.CompilerParams(
            dimension_semantics=("arbitrary", "arbitrary"),
            vmem_limit_bytes=100 * 1024 * 1024,
        ),
    )(A_x, _t(A_k_cache), _t(A_v_cache), A_wq, A_wo,
      B_x, _t(B_k_cache), _t(B_v_cache), B_wq, B_wo)
```

```python
import functools

import jax
import jax.numpy as jnp
import jax.experimental.pallas as pl
import jax.experimental.pallas.tpu as pltpu

HPS = 8
NBUF = 4
PD = 3


def _t(a):
    return jnp.swapaxes(a, 2, 3)


def _qk(q, kt):
    return jnp.dot(q, kt, preferred_element_type=jnp.float32)


def _softmax_pv(s, vt):
    m = jnp.max(s, axis=-1, keepdims=True)
    p = jnp.exp2(s - m)
    l = jnp.sum(p, axis=-1, keepdims=True)
    ot = jax.lax.dot_general(
        vt, p.astype(jnp.bfloat16), (((1,), (1,)), ((), ())),
        preferred_element_type=jnp.float32,
    )
    return (ot.T * (1.0 / l)).astype(jnp.bfloat16)


def _kernel(xa_ref, ka_hbm, va_hbm, wqa_hbm, woa_hbm,
            xb_ref, kb_hbm, vb_hbm, wqb_hbm, wob_hbm,
            o_ref, acc_ref, wqa_ref, woa_ref, wqb_ref, wob_ref,
            kbuf, vbuf, wsems, ksems, vsems,
            *, dh, d, scale, nb, nh):
    b = pl.program_id(0)
    h = pl.program_id(1)
    w = HPS * dh
    nc = 2 * HPS
    assert nc % NBUF == 0 and PD < NBUF

    def w_copies(i):
        cols = pl.ds(i * w, w)
        return [
            pltpu.make_async_copy(wqa_hbm.at[:, cols], wqa_ref.at[:, cols], wsems.at[0, i]),
            pltpu.make_async_copy(wqb_hbm.at[:, cols], wqb_ref.at[:, cols], wsems.at[1, i]),
            pltpu.make_async_copy(woa_hbm.at[cols, :], woa_ref.at[cols, :], wsems.at[2, i]),
            pltpu.make_async_copy(wob_hbm.at[cols, :], wob_ref.at[cols, :], wsems.at[3, i]),
        ]

    def kv_copy(which, bb, hh, c):
        blk, j = divmod(c, HPS)
        src = ((ka_hbm, kb_hbm), (va_hbm, vb_hbm))[which][blk]
        dst = (kbuf, vbuf)[which]
        sem = (ksems, vsems)[which]
        slot = c % NBUF
        return pltpu.make_async_copy(src.at[bb, hh * HPS + j], dst.at[slot], sem.at[slot])

    first = jnp.logical_and(b == 0, h == 0)

    @pl.when(first)
    def _():
        cps = w_copies(0)
        cps[0].start()
        for c in range(PD):
            kv_copy(0, 0, 0, c).start()
            kv_copy(1, 0, 0, c).start()
        for cp in cps[1:]:
            cp.start()
        for i in range(1, nh):
            for cp in w_copies(i):
                cp.start()

    @pl.when(h == 0)
    def _():
        acc_ref[...] = jnp.zeros_like(acc_ref)

    for i in range(nh):
        @pl.when(jnp.logical_and(b == 0, h == i))
        def _():
            for cp in w_copies(i):
                cp.wait()

    wrap = h + 1 == nh
    h_nxt = jnp.where(wrap, 0, h + 1)
    b_nxt = jnp.where(wrap, b + 1, b)
    has_nxt = b_nxt < nb
    b_nxt = jnp.minimum(b_nxt, nb - 1)

    def prefetch(c):
        t = c + PD
        if t < nc:
            kv_copy(0, b, h, t).start()
            kv_copy(1, b, h, t).start()
        else:
            @pl.when(has_nxt)
            def _():
                kv_copy(0, b_nxt, h_nxt, t - nc).start()
                kv_copy(1, b_nxt, h_nxt, t - nc).start()

    off = pl.multiple_of(h * w, 128)
    xs = (xa_ref, xb_ref)
    wqs = (wqa_ref, wqb_ref)
    wos = (woa_ref, wob_ref)
    qs = []
    for blk in range(2):
        q2 = jnp.dot(xs[blk][0], wqs[blk][:, pl.ds(off, w)],
                     preferred_element_type=jnp.float32)
        qs.append((q2 * scale).astype(jnp.bfloat16))

    def qk(c):
        blk, j = divmod(c, HPS)
        kv_copy(0, b, h, c).wait()
        return _qk(qs[blk][:, j * dh:(j + 1) * dh], kbuf[c % NBUF])

    os = [[], []]
    s_next = qk(0)
    for c in range(nc):
        blk, j = divmod(c, HPS)
        prefetch(c)
        s = s_next
        if c + 1 < nc:
            s_next = qk(c + 1)
        kv_copy(1, b, h, c).wait()
        os[blk].append(_softmax_pv(s, vbuf[c % NBUF]))
        if j == HPS - 1:
            o2 = jnp.concatenate(os[blk], axis=-1)
            y = jnp.dot(o2, wos[blk][pl.ds(off, w), :],
                        preferred_element_type=jnp.float32)
            acc_ref[:, blk * d:(blk + 1) * d] += y

    @pl.when(h == nh - 1)
    def _():
        o_ref[0] = acc_ref[...].astype(o_ref.dtype)


@jax.jit
def pallas_concat_heads__gqa_block_cached__gqa_block_cached__near_ridge_kernel(
    A_x: jax.Array,
    A_k_cache: jax.Array,
    A_v_cache: jax.Array,
    A_wq: jax.Array,
    A_wo: jax.Array,
    B_x: jax.Array,
    B_k_cache: jax.Array,
    B_v_cache: jax.Array,
    B_wq: jax.Array,
    B_wo: jax.Array,
):
    B, Sq, D = A_x.shape
    _, H, Sk, Dh = A_k_cache.shape
    nh = H // HPS
    scale = float(Dh) ** -0.5 * 1.4426950408889634

    x_spec = pl.BlockSpec((1, Sq, D), lambda b, h: (b, 0, 0))
    any_spec = pl.BlockSpec(memory_space=pl.ANY)
    specs = [x_spec, any_spec, any_spec, any_spec, any_spec]

    return pl.pallas_call(
        functools.partial(_kernel, dh=Dh, d=D, scale=scale, nb=B, nh=nh),
        grid=(B, nh),
        in_specs=specs + specs,
        out_specs=pl.BlockSpec((1, Sq, 2 * D), lambda b, h: (b, 0, 0)),
        out_shape=jax.ShapeDtypeStruct((B, Sq, 2 * D), jnp.bfloat16),
        scratch_shapes=[
            pltpu.VMEM((Sq, 2 * D), jnp.float32),
            pltpu.VMEM((D, H * Dh), jnp.bfloat16),
            pltpu.VMEM((H * Dh, D), jnp.bfloat16),
            pltpu.VMEM((D, H * Dh), jnp.bfloat16),
            pltpu.VMEM((H * Dh, D), jnp.bfloat16),
            pltpu.VMEM((NBUF, Dh, Sk), jnp.bfloat16),
            pltpu.VMEM((NBUF, Dh, Sk), jnp.bfloat16),
            pltpu.SemaphoreType.DMA((4, nh)),
            pltpu.SemaphoreType.DMA((NBUF,)),
            pltpu.SemaphoreType.DMA((NBUF,)),
        ],
        compiler_params=pltpu.CompilerParams(
            dimension_semantics=("arbitrary", "arbitrary"),
            vmem_limit_bytes=100 * 1024 * 1024,
        ),
    )(A_x, _t(A_k_cache), _t(A_v_cache), A_wq, A_wo,
      B_x, _t(B_k_cache), _t(B_v_cache), B_wq, B_wo)
```

```python
import functools

import jax
import jax.numpy as jnp
import jax.experimental.pallas as pl
import jax.experimental.pallas.tpu as pltpu

HPS = 8


def _t(a):
    return jnp.swapaxes(a, 2, 3)


def _qk(q, kt):
    return jnp.dot(q, kt, preferred_element_type=jnp.float32)


def _softmax_pv(s, vt):
    m = jnp.max(s, axis=-1, keepdims=True)
    p = jnp.exp2(s - m)
    l = jnp.sum(p, axis=-1, keepdims=True)
    ot = jax.lax.dot_general(
        vt, p.astype(jnp.bfloat16), (((1,), (1,)), ((), ())),
        preferred_element_type=jnp.float32,
    )
    return (ot.T * (1.0 / l)).astype(jnp.bfloat16)


def _kernel(xa_ref, ka_ref, va_ref, wqa_hbm, woa_hbm,
            xb_ref, kb_ref, vb_ref, wqb_hbm, wob_hbm,
            o_ref, acc_ref, wqa_ref, woa_ref, wqb_ref, wob_ref, sems,
            *, dh, d, scale, nh):
    b = pl.program_id(0)
    h = pl.program_id(1)
    w = HPS * dh

    def w_copies(i):
        cols = pl.ds(i * w, w)
        return [
            pltpu.make_async_copy(wqa_hbm.at[:, cols], wqa_ref.at[:, cols], sems.at[0, i]),
            pltpu.make_async_copy(wqb_hbm.at[:, cols], wqb_ref.at[:, cols], sems.at[1, i]),
            pltpu.make_async_copy(woa_hbm.at[cols, :], woa_ref.at[cols, :], sems.at[2, i]),
            pltpu.make_async_copy(wob_hbm.at[cols, :], wob_ref.at[cols, :], sems.at[3, i]),
        ]

    @pl.when(jnp.logical_and(b == 0, h == 0))
    def _():
        for i in range(nh):
            for cp in w_copies(i):
                cp.start()

    @pl.when(h == 0)
    def _():
        acc_ref[...] = jnp.zeros_like(acc_ref)

    for i in range(nh):
        @pl.when(jnp.logical_and(b == 0, h == i))
        def _():
            for cp in w_copies(i):
                cp.wait()

    off = pl.multiple_of(h * w, 128)
    blocks = ((xa_ref, ka_ref, va_ref, wqa_ref, woa_ref),
              (xb_ref, kb_ref, vb_ref, wqb_ref, wob_ref))
    qs = []
    for (x_ref, k_ref, v_ref, wq_ref, wo_ref) in blocks:
        q2 = jnp.dot(x_ref[0], wq_ref[:, pl.ds(off, w)],
                     preferred_element_type=jnp.float32)
        qs.append((q2 * scale).astype(jnp.bfloat16))

    chains = [(blk, j) for j in range(HPS) for blk in range(2)]

    def qk(c):
        blk, j = chains[c]
        return _qk(qs[blk][:, j * dh:(j + 1) * dh], blocks[blk][1][0, j])

    os = [[], []]
    s_next = qk(0)
    for c, (blk, j) in enumerate(chains):
        s = s_next
        if c + 1 < len(chains):
            s_next = qk(c + 1)
        os[blk].append(_softmax_pv(s, blocks[blk][2][0, j]))
        if j == HPS - 1:
            o2 = jnp.concatenate(os[blk], axis=-1)
            y = jnp.dot(o2, blocks[blk][4][pl.ds(off, w), :],
                        preferred_element_type=jnp.float32)
            acc_ref[:, blk * d:(blk + 1) * d] += y

    @pl.when(h == nh - 1)
    def _():
        o_ref[0] = acc_ref[...].astype(o_ref.dtype)


@jax.jit
def pallas_concat_heads__gqa_block_cached__gqa_block_cached__near_ridge_kernel(
    A_x: jax.Array,
    A_k_cache: jax.Array,
    A_v_cache: jax.Array,
    A_wq: jax.Array,
    A_wo: jax.Array,
    B_x: jax.Array,
    B_k_cache: jax.Array,
    B_v_cache: jax.Array,
    B_wq: jax.Array,
    B_wo: jax.Array,
):
    B, Sq, D = A_x.shape
    _, H, Sk, Dh = A_k_cache.shape
    nh = H // HPS
    scale = float(Dh) ** -0.5 * 1.4426950408889634

    x_spec = pl.BlockSpec((1, Sq, D), lambda b, h: (b, 0, 0))
    kv_spec = pl.BlockSpec((1, HPS, Dh, Sk), lambda b, h: (b, h, 0, 0))
    w_spec = pl.BlockSpec(memory_space=pl.ANY)
    specs = [x_spec, kv_spec, kv_spec, w_spec, w_spec]

    return pl.pallas_call(
        functools.partial(_kernel, dh=Dh, d=D, scale=scale, nh=nh),
        grid=(B, nh),
        in_specs=specs + specs,
        out_specs=pl.BlockSpec((1, Sq, 2 * D), lambda b, h: (b, 0, 0)),
        out_shape=jax.ShapeDtypeStruct((B, Sq, 2 * D), jnp.bfloat16),
        scratch_shapes=[
            pltpu.VMEM((Sq, 2 * D), jnp.float32),
            pltpu.VMEM((D, H * Dh), jnp.bfloat16),
            pltpu.VMEM((H * Dh, D), jnp.bfloat16),
            pltpu.VMEM((D, H * Dh), jnp.bfloat16),
            pltpu.VMEM((H * Dh, D), jnp.bfloat16),
            pltpu.SemaphoreType.DMA((4, nh)),
        ],
        compiler_params=pltpu.CompilerParams(
            dimension_semantics=("arbitrary", "arbitrary"),
            vmem_limit_bytes=100 * 1024 * 1024,
        ),
    )(A_x, _t(A_k_cache), _t(A_v_cache), A_wq, A_wo,
      B_x, _t(B_k_cache), _t(B_v_cache), B_wq, B_wo)
```

```python
import functools

import jax
import jax.numpy as jnp
import jax.experimental.pallas as pl
import jax.experimental.pallas.tpu as pltpu

HPS = 8


def _t(a):
    return jnp.swapaxes(a, 2, 3)


def _qk(q, kt):
    return jnp.dot(q, kt, preferred_element_type=jnp.float32)


def _softmax_pv_rows(s, vt):
    m = jnp.max(s, axis=-1, keepdims=True)
    p = jnp.exp2(s - m)
    l = jnp.sum(p, axis=-1, keepdims=True)
    ot = jax.lax.dot_general(
        vt, p.astype(jnp.bfloat16), (((1,), (1,)), ((), ())),
        preferred_element_type=jnp.float32,
    )
    return (ot.T * (1.0 / l)).astype(jnp.bfloat16)


def _softmax_pv(s, vt):
    n = s.shape[0]
    parts = [_softmax_pv_rows(s[r:min(r + 128, n)], vt) for r in range(0, n, 128)]
    return jnp.concatenate(parts, axis=0)


def _kernel(xa_ref, ka_ref, va_ref, wqa_hbm, woa_hbm,
            xb_ref, kb_ref, vb_ref, wqb_hbm, wob_hbm,
            o_ref, acc_ref, wqa_ref, woa_ref, wqb_ref, wob_ref, sems,
            *, dh, d, scale, nh):
    b = pl.program_id(0)
    h = pl.program_id(1)
    w = HPS * dh

    def w_copies(i):
        cols = pl.ds(i * w, w)
        return [
            pltpu.make_async_copy(wqa_hbm.at[:, cols], wqa_ref.at[:, cols], sems.at[0, i]),
            pltpu.make_async_copy(wqb_hbm.at[:, cols], wqb_ref.at[:, cols], sems.at[1, i]),
            pltpu.make_async_copy(woa_hbm.at[cols, :], woa_ref.at[cols, :], sems.at[2, i]),
            pltpu.make_async_copy(wob_hbm.at[cols, :], wob_ref.at[cols, :], sems.at[3, i]),
        ]

    @pl.when(jnp.logical_and(b == 0, h == 0))
    def _():
        for i in range(nh):
            for cp in w_copies(i):
                cp.start()

    @pl.when(h == 0)
    def _():
        acc_ref[...] = jnp.zeros_like(acc_ref)

    for i in range(nh):
        @pl.when(jnp.logical_and(b == 0, h == i))
        def _():
            for cp in w_copies(i):
                cp.wait()

    off = pl.multiple_of(h * w, 128)
    blocks = ((xa_ref, ka_ref, va_ref, wqa_ref, woa_ref),
              (xb_ref, kb_ref, vb_ref, wqb_ref, wob_ref))
    qs = []
    for (x_ref, k_ref, v_ref, wq_ref, wo_ref) in blocks:
        q2 = jnp.dot(x_ref[0], wq_ref[:, pl.ds(off, w)],
                     preferred_element_type=jnp.float32)
        qs.append((q2 * scale).astype(jnp.bfloat16))

    chains = [(blk, j) for blk in range(2) for j in range(HPS)]

    def qk(c):
        blk, j = chains[c]
        return _qk(qs[blk][:, j * dh:(j + 1) * dh], blocks[blk][1][0, j])

    os = [[], []]
    s_next = qk(0)
    for c, (blk, j) in enumerate(chains):
        s = s_next
        if c + 1 < len(chains):
            s_next = qk(c + 1)
        os[blk].append(_softmax_pv(s, blocks[blk][2][0, j]))
        if j == HPS - 1:
            o2 = jnp.concatenate(os[blk], axis=-1)
            y = jnp.dot(o2, blocks[blk][4][pl.ds(off, w), :],
                        preferred_element_type=jnp.float32)
            acc_ref[:, blk * d:(blk + 1) * d] += y

    @pl.when(h == nh - 1)
    def _():
        o_ref[0] = acc_ref[...].astype(o_ref.dtype)


@jax.jit
def pallas_concat_heads__gqa_block_cached__gqa_block_cached__near_ridge_kernel(
    A_x: jax.Array,
    A_k_cache: jax.Array,
    A_v_cache: jax.Array,
    A_wq: jax.Array,
    A_wo: jax.Array,
    B_x: jax.Array,
    B_k_cache: jax.Array,
    B_v_cache: jax.Array,
    B_wq: jax.Array,
    B_wo: jax.Array,
):
    B, Sq, D = A_x.shape
    _, H, Sk, Dh = A_k_cache.shape
    nh = H // HPS
    scale = float(Dh) ** -0.5 * 1.4426950408889634

    x_spec = pl.BlockSpec((1, Sq, D), lambda b, h: (b, 0, 0))
    kv_spec = pl.BlockSpec((1, HPS, Dh, Sk), lambda b, h: (b, h, 0, 0))
    w_spec = pl.BlockSpec(memory_space=pl.ANY)
    specs = [x_spec, kv_spec, kv_spec, w_spec, w_spec]

    return pl.pallas_call(
        functools.partial(_kernel, dh=Dh, d=D, scale=scale, nh=nh),
        grid=(B, nh),
        in_specs=specs + specs,
        out_specs=pl.BlockSpec((1, Sq, 2 * D), lambda b, h: (b, 0, 0)),
        out_shape=jax.ShapeDtypeStruct((B, Sq, 2 * D), jnp.bfloat16),
        scratch_shapes=[
            pltpu.VMEM((Sq, 2 * D), jnp.float32),
            pltpu.VMEM((D, H * Dh), jnp.bfloat16),
            pltpu.VMEM((H * Dh, D), jnp.bfloat16),
            pltpu.VMEM((D, H * Dh), jnp.bfloat16),
            pltpu.VMEM((H * Dh, D), jnp.bfloat16),
            pltpu.SemaphoreType.DMA((4, nh)),
        ],
        compiler_params=pltpu.CompilerParams(
            dimension_semantics=("arbitrary", "arbitrary"),
            vmem_limit_bytes=100 * 1024 * 1024,
        ),
    )(A_x, _t(A_k_cache), _t(A_v_cache), A_wq, A_wo,
      B_x, _t(B_k_cache), _t(B_v_cache), B_wq, B_wo)
```

```python
import functools

import jax
import jax.numpy as jnp
import jax.experimental.pallas as pl
import jax.experimental.pallas.tpu as pltpu

HPS = 8


def _t(a):
    return jnp.swapaxes(a, 2, 3)


def _qk(q, kt):
    return jnp.dot(q, kt, preferred_element_type=jnp.float32)


def _softmax_pv(s, vt):
    m = jnp.max(s, axis=-1, keepdims=True)
    p = jnp.exp2(s - m)
    l = jnp.sum(p, axis=-1, keepdims=True)
    ot = jax.lax.dot_general(
        vt, p.astype(jnp.bfloat16), (((1,), (1,)), ((), ())),
        preferred_element_type=jnp.float32,
    )
    return (ot.T * (1.0 / l)).astype(jnp.bfloat16)


def _kernel(xa_ref, ka_ref, va_ref, wqa_hbm, woa_hbm,
            xb_ref, kb_ref, vb_ref, wqb_hbm, wob_hbm,
            o_ref, acc_ref, wqa_ref, woa_ref, wqb_ref, wob_ref, sems,
            *, dh, d, scale, nh):
    b = pl.program_id(0)
    h = pl.program_id(1)
    w = HPS * dh

    def w_copies(i):
        cols = pl.ds(i * w, w)
        return [
            pltpu.make_async_copy(wqa_hbm.at[:, cols], wqa_ref.at[:, cols], sems.at[0, i]),
            pltpu.make_async_copy(wqb_hbm.at[:, cols], wqb_ref.at[:, cols], sems.at[1, i]),
            pltpu.make_async_copy(woa_hbm.at[cols, :], woa_ref.at[cols, :], sems.at[2, i]),
            pltpu.make_async_copy(wob_hbm.at[cols, :], wob_ref.at[cols, :], sems.at[3, i]),
        ]

    @pl.when(jnp.logical_and(b == 0, h == 0))
    def _():
        for i in range(nh):
            for cp in w_copies(i):
                cp.start()

    @pl.when(h == 0)
    def _():
        acc_ref[...] = jnp.zeros_like(acc_ref)

    for i in range(nh):
        @pl.when(jnp.logical_and(b == 0, h == i))
        def _():
            for cp in w_copies(i):
                cp.wait()

    off = pl.multiple_of(h * w, 128)
    blocks = ((xa_ref, ka_ref, va_ref, wqa_ref, woa_ref),
              (xb_ref, kb_ref, vb_ref, wqb_ref, wob_ref))
    qs = []
    for (x_ref, k_ref, v_ref, wq_ref, wo_ref) in blocks:
        q2 = jnp.dot(x_ref[0], wq_ref[:, pl.ds(off, w)],
                     preferred_element_type=jnp.float32)
        qs.append((q2 * scale).astype(jnp.bfloat16))

    chains = [(blk, j) for blk in range(2) for j in range(HPS)]

    def qk(c):
        blk, j = chains[c]
        return _qk(qs[blk][:, j * dh:(j + 1) * dh], blocks[blk][1][0, j])

    os = [[], []]
    s_next = qk(0)
    for c, (blk, j) in enumerate(chains):
        s = s_next
        if c + 1 < len(chains):
            s_next = qk(c + 1)
        os[blk].append(_softmax_pv(s, blocks[blk][2][0, j]))
        if j == HPS - 1:
            o2 = jnp.concatenate(os[blk], axis=-1)
            y = jnp.dot(o2, blocks[blk][4][pl.ds(off, w), :],
                        preferred_element_type=jnp.float32)
            acc_ref[:, blk * d:(blk + 1) * d] += y

    @pl.when(h == nh - 1)
    def _():
        o_ref[0] = acc_ref[...].astype(o_ref.dtype)


@jax.jit
def pallas_concat_heads__gqa_block_cached__gqa_block_cached__near_ridge_kernel(
    A_x: jax.Array,
    A_k_cache: jax.Array,
    A_v_cache: jax.Array,
    A_wq: jax.Array,
    A_wo: jax.Array,
    B_x: jax.Array,
    B_k_cache: jax.Array,
    B_v_cache: jax.Array,
    B_wq: jax.Array,
    B_wo: jax.Array,
):
    B, Sq, D = A_x.shape
    _, H, Sk, Dh = A_k_cache.shape
    nh = H // HPS
    scale = float(Dh) ** -0.5 * 1.4426950408889634

    x_spec = pl.BlockSpec((1, Sq, D), lambda b, h: (b, 0, 0))
    kv_spec = pl.BlockSpec((1, HPS, Dh, Sk), lambda b, h: (b, h, 0, 0))
    w_spec = pl.BlockSpec(memory_space=pl.ANY)
    specs = [x_spec, kv_spec, kv_spec, w_spec, w_spec]

    return pl.pallas_call(
        functools.partial(_kernel, dh=Dh, d=D, scale=scale, nh=nh),
        grid=(B, nh),
        in_specs=specs + specs,
        out_specs=pl.BlockSpec((1, Sq, 2 * D), lambda b, h: (b, 0, 0)),
        out_shape=jax.ShapeDtypeStruct((B, Sq, 2 * D), jnp.bfloat16),
        scratch_shapes=[
            pltpu.VMEM((Sq, 2 * D), jnp.float32),
            pltpu.VMEM((D, H * Dh), jnp.bfloat16),
            pltpu.VMEM((H * Dh, D), jnp.bfloat16),
            pltpu.VMEM((D, H * Dh), jnp.bfloat16),
            pltpu.VMEM((H * Dh, D), jnp.bfloat16),
            pltpu.SemaphoreType.DMA((4, nh)),
        ],
        compiler_params=pltpu.CompilerParams(
            dimension_semantics=("arbitrary", "arbitrary"),
            vmem_limit_bytes=100 * 1024 * 1024,
        ),
    )(A_x, _t(A_k_cache), _t(A_v_cache), A_wq, A_wo,
      B_x, _t(B_k_cache), _t(B_v_cache), B_wq, B_wo)
```
